```python
import os as _os
_os.environ.setdefault("JAX_PLATFORMS", "cpu")
import jax
import jax.numpy as jnp

def _softmax(x, axis=-1):
    return jax.nn.softmax(x, axis=axis)
def _gelu(x):
    return jax.nn.gelu(x, approximate=True)
def _silu(x):
    return jax.nn.silu(x)
def _sigmoid(x):
    return jax.nn.sigmoid(x)
def _layernorm(x, axis=-1, eps=1e-5):
    m = jnp.mean(x, axis=axis, keepdims=True)
    v = jnp.var(x, axis=axis, keepdims=True)
    return (x - m) / jnp.sqrt(v + eps)
def _scatter_add(tgt, idx, src, axis=0):
    return tgt.at[idx].add(src)
def _segment_sum(src, seg, n):
    return jax.ops.segment_sum(src, seg, n)
class _Rng:
    def __init__(self, key):
        self._k = key
    def _next(self):
        self._k, sub = jax.random.split(self._k)
        return sub
    def normal(self, shape):
        return jax.random.normal(self._next(), shape, dtype=jnp.bfloat16)
    def randint(self, lo, hi, shape):
        return jax.random.randint(self._next(), shape, lo, hi, dtype=jnp.int32)
    def uniform(self, shape, lo=0.0, hi=1.0):
        return jax.random.uniform(self._next(), shape, jnp.bfloat16, lo, hi)
    def permutation(self, n):
        return jax.random.permutation(self._next(), n)


kernel_name = 'standalone__mha_block_cached__near_ridge'

def setup_inputs():
    _rng = _Rng(jax.random.key(int.from_bytes(__import__("os").urandom(4), "little")))
    _w = (lambda a: (lambda t: t.astype(jnp.bfloat16) if jnp.issubdtype(t.dtype, jnp.floating) else t)(jnp.asarray(a)))
    B, Sq, D = 8, 96, 576
    H, Sk, Dh = 32, 96, 128
    return {
        "x": _w((lambda *s: _rng.normal(s) * 0.8)(B, Sq, D)),
        "k_cache": _w((lambda *s: _rng.normal(s) * 0.8)(B, H, Sk, Dh)),
        "v_cache": _w((lambda *s: _rng.normal(s) * 0.05)(B, H, Sk, Dh)),
        "wq": _w((lambda *s: _rng.normal(s) * 0.8)(D, H * Dh) * (D ** -0.5)),
        "wo": _w((lambda *s: _rng.normal(s) * 0.05)(H * Dh, D) * ((H * Dh) ** -0.5)),
    }

def reference(x, k_cache, v_cache, wq, wo):
    B, Sq, D = x.shape
    H, Dh = 32, 128
    q = (lambda x, *d: x.transpose(*d))((x @ wq).reshape(B, Sq, H, Dh), 0, 2, 1, 3)
    scores = jnp.einsum("bhqd,bhkd->bhqk", q, k_cache) * (Dh ** -0.5)
    p = _softmax(scores, axis=-1)
    o = jnp.einsum("bhqk,bhkd->bhqd", p, v_cache)
    return (lambda x, *d: x.transpose(*d))(o, 0, 2, 1, 3).reshape(B, Sq, H * Dh) @ wo
```

```python
import functools
import math
import jax
import jax.numpy as jnp
from jax import lax
import jax.experimental.pallas as pl
import jax.experimental.pallas.tpu as pltpu

NT = (((1,), (1,)), ((), ()))
G = 4
XC = 4
OC = 3


def _kernel(x_hbm, k_hbm, v_hbm, wq_hbm, wo_hbm, out_hbm,
            x_v, k_v, v_v, wq_v, wo_v, qt_v, q_v, oh_v, acc_v, tail_v, out_v, sem,
            *, B, Sq, D, H, Dh, c):
    NG = H // G
    W = G * Dh
    M = B * Sq
    DM = (D // 128) * 128
    NJ = DM // 128
    NTT = M // 128
    XR = M // XC
    OR = M // OC
    f32 = jnp.float32
    bf = jnp.bfloat16

    S_OUT = XC + 1 + NG

    def cp_x(ci, s):
        return pltpu.make_async_copy(x_hbm.at[pl.ds(ci * XR, XR)], x_v.at[pl.ds(ci * XR, XR)], sem.at[s])
    def cp_wq(g, s):
        return pltpu.make_async_copy(wq_hbm.at[:, pl.ds(g * W, W)], wq_v.at[g], sem.at[s])
    def cp_wo(g, s):
        return pltpu.make_async_copy(wo_hbm.at[:, pl.ds(g * W, W)], wo_v.at[g], sem.at[s])
    def cp_k(g, s):
        return pltpu.make_async_copy(k_hbm.at[:, pl.ds(g * G, G)], k_v.at[:, pl.ds(g * G, G)], sem.at[s])
    def cp_v(g, s):
        return pltpu.make_async_copy(v_hbm.at[:, pl.ds(g * G, G)], v_v.at[:, pl.ds(g * G, G)], sem.at[s])
    def cp_out(ci):
        return pltpu.make_async_copy(out_v.at[pl.ds(ci * OR, OR)], out_hbm.at[pl.ds(ci * OR, OR)], sem.at[S_OUT])

    def set_copies(g, last):
        s = XC + 1 + g
        cps = []
        if not last:
            cps.append(cp_wq(g + 1, s))
        cps += [cp_k(g, s), cp_v(g, s), cp_wo(g - 1, s)]
        if last:
            cps.append(cp_wo(g, s))
        return cps

    cp_wq(0, 0).start()
    for ci in range(XC):
        cp_x(ci, ci).start()
    cp_wq(1, XC).start()
    cp_k(0, XC + 1).start()
    cp_v(0, XC + 1).start()
    for g in range(1, NG):
        for cp in set_copies(g, g == NG - 1):
            cp.start()

    def Qtail(g, rows):
        qt_v[rows, :] = jnp.dot(x_v[rows, DM:D], wq_v[g, DM:D, :], preferred_element_type=f32)

    def Qmain(g, j, rows):
        q = jnp.dot(x_v[rows, 0:DM], wq_v[g, 0:DM, j * Dh:(j + 1) * Dh], preferred_element_type=f32)
        q = q + qt_v[rows, j * Dh:(j + 1) * Dh]
        q_v[rows, j * Dh:(j + 1) * Dh] = q.astype(bf)

    def QK(g, i, qc):
        j = i // 2
        res = []
        for b in range(4 * (i % 2), 4 * (i % 2) + 4):
            qbh = qc[b * Sq:(b + 1) * Sq, j * Dh:(j + 1) * Dh]
            s = lax.dot_general(qbh, k_v[b, g * G + j], NT, preferred_element_type=f32)
            m = jnp.max(s, axis=-1, keepdims=True)
            p = jnp.exp2((s - m) * c)
            l = jnp.sum(p, axis=-1, keepdims=True)
            res.append((p.astype(bf), pl.reciprocal(l, approx=True)))
        return res

    def PV(g, i, res):
        j = i // 2
        for n, b in enumerate(range(4 * (i % 2), 4 * (i % 2) + 4)):
            p, rl = res[n]
            o = jnp.dot(p, v_v[b, g * G + j], preferred_element_type=f32)
            oh_v[b * Sq:(b + 1) * Sq, j * Dh:(j + 1) * Dh] = (o * rl).astype(bf)

    def Omain(g, j, rows, ohp):
        part = lax.dot_general(ohp[rows, :], wo_v[g, j * 128:(j + 1) * 128, :], NT, preferred_element_type=f32)
        acc_v[rows, j * 128:(j + 1) * 128] += part

    def Otail(g, t, ohp):
        part = lax.dot_general(wo_v[g, DM:D, :], ohp[t * 128:(t + 1) * 128, :], NT, preferred_element_type=f32)
        tail_v[t] += part

    ALL = slice(0, M)
    H0, H1 = slice(0, M // 2), slice(M // 2, M)

    def attn_stage(g, qc, fillers, small):
        nf = len(fillers)
        res = None
        for i in range(8):
            if res is not None:
                PV(g, i - 1, res)
            res = QK(g, i, qc)
            lo = (i * nf) // 9; hi = ((i + 1) * nf) // 9
            for f in fillers[lo:hi]: f()
            if small: small.pop(0)()
        PV(g, 7, res)
        for f in fillers[(8 * nf) // 9:]: f()
        for f in small: f()

    acc_v[...] = jnp.zeros_like(acc_v)
    tail_v[...] = jnp.zeros_like(tail_v)
    cp_wq(0, 0).wait()

    def p1_body(ci, carry):
        cp_x(ci, ci).wait()
        rows = pl.ds(pl.multiple_of(ci * XR, XR), XR)
        Qtail(0, rows)
        for j in range(G): Qmain(0, j, rows)
        return carry
    lax.fori_loop(0, XC, p1_body, 0)

    cp_wq(1, XC).wait()
    qc = q_v[...]
    Qtail(1, ALL)
    Qmain(1, 0, ALL)
    cp_k(0, XC + 1).wait()
    cp_v(0, XC + 1).wait()
    T3 = [slice(0, 256), slice(256, 512), slice(512, 768)]
    fill = [functools.partial(Qmain, 1, j, r) for j in range(1, G) for r in T3]
    attn_stage(0, qc, fill, [])

    def body(g, carry):
        for cp in set_copies(g, False):
            cp.wait()
        qc = q_v[...]
        ohp = oh_v[...]
        fill = [functools.partial(Qtail, g + 1, ALL)]
        fill += [functools.partial(Qmain, g + 1, j, ALL) for j in range(G)]
        fill += [functools.partial(Omain, g - 1, j, ALL, ohp) for j in range(NJ)]
        small = [functools.partial(Otail, g - 1, t, ohp) for t in range(NTT)]
        attn_stage(g, qc, fill, small)
        return carry
    lax.fori_loop(1, NG - 1, body, 0)

    gl = NG - 1
    for cp in set_copies(gl, True):
        cp.wait()
    qc = q_v[...]
    ohp = oh_v[...]
    fill = [functools.partial(Omain, gl - 1, j, r, ohp) for j in range(NJ) for r in (H0, H1)]
    small = [functools.partial(Otail, gl - 1, t, ohp) for t in range(NTT)]
    fill.append(small.pop())
    attn_stage(gl, qc, fill, small)

    TPC = OR // 128
    def e2_body(ci, carry):
        r0 = pl.multiple_of(ci * OR, OR)
        rows = pl.ds(r0, OR)
        ohc = oh_v[rows, :]
        for tt in range(TPC):
            t = ci * TPC + tt
            trow = pl.ds(pl.multiple_of(r0 + tt * 128, 128), 128)
            part = lax.dot_general(wo_v[gl, DM:D, :], ohc[tt * 128:(tt + 1) * 128, :], NT, preferred_element_type=f32)
            out_v[trow, DM:D] = (tail_v[t] + part).T.astype(bf)
        for j in range(NJ):
            part = lax.dot_general(ohc, wo_v[gl, j * 128:(j + 1) * 128, :], NT,
                                   preferred_element_type=f32)
            out_v[rows, j * 128:(j + 1) * 128] = (acc_v[rows, j * 128:(j + 1) * 128] + part).astype(bf)
        cp_out(ci).start()
        return carry
    lax.fori_loop(0, OC, e2_body, 0)
    for ci in range(OC):
        cp_out(ci).wait()


@jax.jit
def pallas_standalone__mha_block_cached__near_ridge_kernel(x, k_cache, v_cache, wq, wo):
    B, Sq, D = x.shape
    _, H, Sk, Dh = k_cache.shape
    M = B * Sq
    NG = H // G
    x2 = x.reshape(M, D)
    kern = functools.partial(_kernel, B=B, Sq=Sq, D=D, H=H, Dh=Dh, c=Dh ** -0.5 * math.log2(math.e))
    bf = jnp.bfloat16
    out = pl.pallas_call(
        kern,
        in_specs=[pl.BlockSpec(memory_space=pl.ANY)] * 5,
        out_specs=pl.BlockSpec(memory_space=pl.ANY),
        out_shape=jax.ShapeDtypeStruct((M, D), x.dtype),
        scratch_shapes=[
            pltpu.VMEM((M, D), bf),
            pltpu.VMEM((B, H, Sk, Dh), bf),
            pltpu.VMEM((B, H, Sk, Dh), bf),
            pltpu.VMEM((NG, D, G * Dh), bf),
            pltpu.VMEM((NG, D, G * Dh), bf),
            pltpu.VMEM((M, G * Dh), jnp.float32),
            pltpu.VMEM((M, G * Dh), bf),
            pltpu.VMEM((M, G * Dh), bf),
            pltpu.VMEM((M, 512), jnp.float32),
            pltpu.VMEM((M // 128, D - 512, 128), jnp.float32),
            pltpu.VMEM((M, D), bf),
            pltpu.SemaphoreType.DMA((XC + 2 + NG,)),
        ],
        compiler_params=pltpu.CompilerParams(
            vmem_limit_bytes=100 * 1024 * 1024,
        ),
    )(x2, k_cache, v_cache, wq, wo.T)
    return out.reshape(B, Sq, D)
```

```python
import functools
import math
import jax
import jax.numpy as jnp
from jax import lax
import jax.experimental.pallas as pl
import jax.experimental.pallas.tpu as pltpu

NT = (((1,), (1,)), ((), ()))
G = 4
NLOOP = 4
P = functools.partial


def _kernel(x_hbm, k_hbm, v_hbm, wq_hbm, wo_hbm, out_hbm,
            x_v, k_v, v_v, wq_v, wo_v, qt_v, q_v, oh_v, acc_v, tail_v, out_v, outt_v, sem,
            *, B, Sq, D, H, Dh, c):
    NG = H // G
    W = G * Dh
    M = B * Sq
    DM = (D // 128) * 128
    NJ = DM // 128
    NTT = M // 128
    XR = M // 4
    f32 = jnp.float32
    bf = jnp.bfloat16

    S_SET = 6
    S_REST = S_SET + NLOOP
    S_OUT = S_REST + 1

    def cp_x(r0, n, s):
        return pltpu.make_async_copy(x_hbm.at[pl.ds(r0, n)], x_v.at[pl.ds(r0, n)], sem.at[s])
    def cp_wq(g, s):
        return pltpu.make_async_copy(wq_hbm.at[:, pl.ds(g * W, W)], wq_v.at[g], sem.at[s])
    def cp_wq_half(hf, s):
        return pltpu.make_async_copy(wq_hbm.at[:, pl.ds(hf * (W // 2), W // 2)],
                                     wq_v.at[0, :, pl.ds(hf * (W // 2), W // 2)], sem.at[s])
    def cp_wo(g, s):
        return pltpu.make_async_copy(wo_hbm.at[:, pl.ds(g * W, W)], wo_v.at[g], sem.at[s])
    def cp_k(g, s, n=1):
        return pltpu.make_async_copy(k_hbm.at[:, pl.ds(g * G, n * G)], k_v.at[:, pl.ds(g * G, n * G)], sem.at[s])
    def cp_v(g, s, n=1):
        return pltpu.make_async_copy(v_hbm.at[:, pl.ds(g * G, n * G)], v_v.at[:, pl.ds(g * G, n * G)], sem.at[s])
    def cp_out(r0, n, c0=0, nc=DM):
        cs = pl.ds(c0, nc)
        return pltpu.make_async_copy(out_v.at[pl.ds(r0, n), cs], out_hbm.at[pl.ds(r0, n), cs], sem.at[S_OUT])
    def cp_outt(r0, n):
        return pltpu.make_async_copy(outt_v.at[pl.ds(r0, n)], out_hbm.at[pl.ds(r0, n), pl.ds(DM, D - DM)],
                                     sem.at[S_OUT])

    def set_copies(g):
        s = S_SET + g - 1
        return [cp_wq(g + 2, s), cp_k(g, s), cp_v(g, s), cp_wo(g - 1, s)]

    g5 = NLOOP + 1
    d0 = [cp_wq_half(0, 0), cp_x(0, XR, 0)]
    d1 = [cp_wq_half(1, 1)]
    d2 = [cp_x(XR, XR, 2)]
    d3 = [cp_x(2 * XR, 2 * XR, 3)]
    d4 = [cp_wq(1, 4)]
    d5 = [cp_wq(2, 5), cp_k(0, 5), cp_v(0, 5)]
    rest = [cp_wq(g, S_REST) for g in range(g5 + 2, NG)]
    rest += [cp_k(g5, S_REST, NG - g5), cp_v(g5, S_REST, NG - g5)]
    rest += [cp_wo(g, S_REST) for g in range(g5 - 1, NG)]
    for cp in d0 + d1 + d2 + d3 + d4 + d5:
        cp.start()
    for g in range(1, NLOOP + 1):
        for cp in set_copies(g):
            cp.start()
    for cp in rest:
        cp.start()

    def wait(cps):
        for cp in cps:
            cp.wait()

    def Qtail(g, rows):
        qt_v[rows, :] = jnp.dot(x_v[rows, DM:D], wq_v[g, DM:D, :], preferred_element_type=f32)

    def Qtail_half(hf, r0, n):
        cs = slice(hf * (W // 2), (hf + 1) * (W // 2))
        for rr in (slice(r0, r0 + n // 2), slice(r0 + n // 2, r0 + n)):
            qt_v[rr, cs] = jnp.dot(x_v[rr, DM:D], wq_v[0, DM:D, cs], preferred_element_type=f32)

    def Qmain(g, j, rows):
        q = jnp.dot(x_v[rows, 0:DM], wq_v[g, 0:DM, j * Dh:(j + 1) * Dh], preferred_element_type=f32)
        q = q + qt_v[rows, j * Dh:(j + 1) * Dh]
        q_v[g, rows, j * Dh:(j + 1) * Dh] = q.astype(bf)

    def QK(g, units, qc):
        res = []
        for b, j in units:
            qbh = qc[b * Sq:(b + 1) * Sq, j * Dh:(j + 1) * Dh]
            s = lax.dot_general(qbh, k_v[b, g * G + j], NT, preferred_element_type=f32)
            m = jnp.max(s, axis=-1, keepdims=True)
            p = jnp.exp2((s - m) * c)
            l = jnp.sum(p, axis=-1, keepdims=True)
            r = pl.reciprocal(l, approx=True)
            r = r * (2.0 - l * r)
            res.append((p * r).astype(bf))
        return res

    def PV(g, units, res, ohw):
        for n, (b, j) in enumerate(units):
            o = jnp.dot(res[n], v_v[b, g * G + j], preferred_element_type=f32)
            ohw[b * Sq:(b + 1) * Sq, j * Dh:(j + 1) * Dh] = o.astype(bf)

    BY_HEAD = [[(b, i // 2) for b in range(4 * (i % 2), 4 * (i % 2) + 4)] for i in range(8)]
    BY_BATCH = [[(b, j) for j in range(G)] for b in range(B)]

    def Omain(g, j, rows, ohp, final=False):
        part = lax.dot_general(ohp[rows, :], wo_v[g, j * 128:(j + 1) * 128, :], NT, preferred_element_type=f32)
        cs = slice(j * 128, (j + 1) * 128)
        if final:
            out_v[rows, cs] = (acc_v[rows, cs] + part).astype(bf)
        else:
            acc_v[rows, cs] += part

    def Otail(g, t, ohp, final=False):
        part = lax.dot_general(wo_v[g, DM:D, :], ohp[t * 128:(t + 1) * 128, :], NT, preferred_element_type=f32)
        if final:
            outt_v[t * 128:(t + 1) * 128, :] = (tail_v[t] + part).T.astype(bf)
        else:
            tail_v[t] += part

    ALL = slice(0, M)
    H0, H1 = slice(0, M // 2), slice(M // 2, M)

    def attn_stage(g, qc, pos, ohw, order=BY_HEAD):
        res = None
        for n, i in enumerate(order):
            if res is not None:
                PV(g, order[n - 1], res, ohw)
            res = QK(g, i, qc)
            for f in pos[n]: f()
        PV(g, order[7], res, ohw)
        for f in pos[8]: f()

    def full_stage(g, qc, ohp, ohw):
        Qtail(g + 2, ALL)
        for j in range(NJ - 1): Omain(g - 1, j, ALL, ohp)
        for t in range(NTT): Otail(g - 1, t, ohp)
        pos = [[P(Omain, g - 1, NJ - 1, ALL, ohp)]]
        pos += [[P(Qmain, g + 2, j, r)] for j in range(G) for r in (H0, H1)]
        attn_stage(g, qc, pos, ohw)

    def zero_body(i, carry):
        acc_v[pl.ds(pl.multiple_of(i * 128, 128), 128), :] = jnp.zeros((128, DM), f32)
        tail_v[i] = jnp.zeros((D - DM, 128), f32)
        return carry
    lax.fori_loop(0, NTT, zero_body, 0)

    R0, R1, R23 = slice(0, XR), slice(XR, 2 * XR), slice(2 * XR, M)
    wait(d0)
    Qtail_half(0, 0, XR); Qmain(0, 0, R0); Qmain(0, 1, R0)
    wait(d1)
    Qtail_half(1, 0, XR); Qmain(0, 2, R0); Qmain(0, 3, R0)
    wait(d2)
    Qtail(0, R1)
    for j in range(G): Qmain(0, j, R1)
    wait(d3)
    Qtail(0, R23)
    for j in range(G): Qmain(0, j, R23)
    wait(d4)
    Qtail(1, ALL)
    for j in range(G): Qmain(1, j, ALL)
    wait(d5)
    Qtail(2, H0)
    hl = [P(Qtail, 2, H1)] + [P(Qmain, 2, j, r) for j in range(G) for r in (H0, H1)]
    attn_stage(0, q_v.at[0], [[f] for f in hl], oh_v.at[0])

    def body(g, carry):
        wait(set_copies(g))
        qc = q_v[g]
        full_stage(g, qc, oh_v.at[0], oh_v.at[0])
        return carry
    lax.fori_loop(1, NLOOP + 1, body, 0)

    wait(rest)
    for g in range(g5, NG - 2):
        full_stage(g, q_v.at[g], oh_v.at[0 if g == g5 else g - 1], oh_v.at[g])
    g = NG - 2
    ohp = oh_v.at[g - 1]
    hl = [P(Omain, g - 1, j, r, ohp) for j in range(NJ) for r in (H0, H1)]
    T = [P(Otail, g - 1, t, ohp) for t in range(NTT)]
    attn_stage(g, q_v.at[g], [[f] for f in hl[:4]] + [T] + [[f] for f in hl[4:]], oh_v.at[g])
    g = NG - 1
    ohp = oh_v.at[g - 1]
    ohl = oh_v.at[g]
    TR = [slice(t * 128, (t + 1) * 128) for t in range(NTT)]
    outs = []
    def emit(*a):
        outs.append(cp_out(*a))
        outs[-1].start()
    def emitt(*a):
        outs.append(cp_outt(*a))
        outs[-1].start()
    def o6(rows, js): return [P(Omain, g - 1, j, rows, ohp) for j in js]
    T6 = [P(Otail, g - 1, t, ohp) for t in range(NTT)]
    def t7(t): return [P(Otail, g, t, ohl, True)]
    def o7(t, js=range(NJ)): return [P(Omain, g, j, TR[t], ohl, True) for j in js]
    pos = [o6(H0, [0, 1]),
           o6(H0, [2]) + T6[:3],
           o6(H0, [3]) + T6[3:],
           t7(0) + o7(0) + [P(emit, 0, 128)],
           t7(1) + o7(1) + [P(emit, 128, 128)],
           t7(2) + o7(2) + [P(emit, 256, 128)],
           o6(H1, [0, 1]),
           o6(H1, [2, 3]) + t7(3) + o7(3) + [P(emit, 384, 128), P(emitt, 0, 256)],
           t7(4) + o7(4) + [P(emit, 512, 128), P(emitt, 256, 256)]]
    attn_stage(g, q_v.at[g], pos, ohl, order=BY_BATCH)
    for f in t7(5) + o7(5, [3, 2, 1]): f()
    emit(640, 128, 128, DM - 128)
    emitt(512, 256)
    for f in o7(5, [0]): f()
    emit(640, 128, 0, 128)
    wait(outs)


@jax.jit
def pallas_standalone__mha_block_cached__near_ridge_kernel(x, k_cache, v_cache, wq, wo):
    B, Sq, D = x.shape
    _, H, Sk, Dh = k_cache.shape
    M = B * Sq
    NG = H // G
    x2 = x.reshape(M, D)
    kern = functools.partial(_kernel, B=B, Sq=Sq, D=D, H=H, Dh=Dh, c=Dh ** -0.5 * math.log2(math.e))
    bf = jnp.bfloat16
    out = pl.pallas_call(
        kern,
        in_specs=[pl.BlockSpec(memory_space=pl.ANY)] * 5,
        out_specs=pl.BlockSpec(memory_space=pl.ANY),
        out_shape=jax.ShapeDtypeStruct((M, D), x.dtype),
        scratch_shapes=[
            pltpu.VMEM((M, D), bf),
            pltpu.VMEM((B, H, Sk, Dh), bf),
            pltpu.VMEM((B, H, Sk, Dh), bf),
            pltpu.VMEM((NG, D, G * Dh), bf),
            pltpu.VMEM((NG, D, G * Dh), bf),
            pltpu.VMEM((M, G * Dh), jnp.float32),
            pltpu.VMEM((NG, M, G * Dh), bf),
            pltpu.VMEM((NG, M, G * Dh), bf),
            pltpu.VMEM((M, 512), jnp.float32),
            pltpu.VMEM((M // 128, D - 512, 128), jnp.float32),
            pltpu.VMEM((M, 512), bf),
            pltpu.VMEM((M, D - 512), bf),
            pltpu.SemaphoreType.DMA((6 + NLOOP + 2,)),
        ],
        compiler_params=pltpu.CompilerParams(
            vmem_limit_bytes=100 * 1024 * 1024,
        ),
    )(x2, k_cache, v_cache, wq, wo.T)
    return out.reshape(B, Sq, D)
```

```python
import functools
import math

import jax
import jax.numpy as jnp
from jax import lax
import jax.experimental.pallas as pl
import jax.experimental.pallas.tpu as pltpu

NT = (((1,), (1,)), ((), ()))
G = 4
NLOOP = 4
NSEM = 6
P = functools.partial


def _kernel(x_hbm, k_hbm, v_hbm, wq_hbm, wo_hbm, out_hbm,
            x_v, k_v, v_v, wq_v, wo_v, qt_v, q_v, oh_v, acc_v, tail_v, out_v, outt_v, sem,
            *, B, Sq, D, H, Dh, c):
    NG = H // G
    W = G * Dh
    M = B * Sq
    DM = (D // 128) * 128
    NJ = DM // 128
    NTT = M // 128
    XR = M // 4
    f32 = jnp.float32
    bf = jnp.bfloat16

    def cp_x(r0, n, s):
        return pltpu.make_async_copy(x_hbm.at[pl.ds(r0, n)], x_v.at[pl.ds(r0, n)], sem.at[s])

    def cp_wq(g, s):
        return pltpu.make_async_copy(wq_hbm.at[:, pl.ds(g * W, W)], wq_v.at[g], sem.at[s])

    def cp_wq_half(hf, s):
        cs = pl.ds(hf * (W // 2), W // 2)
        return pltpu.make_async_copy(wq_hbm.at[:, cs], wq_v.at[0, :, cs], sem.at[s])

    def cp_wo(g, s):
        return pltpu.make_async_copy(wo_hbm.at[:, pl.ds(g * W, W)], wo_v.at[g], sem.at[s])

    def cp_k(g, s, n=1):
        hs = pl.ds(g * G, n * G)
        return pltpu.make_async_copy(k_hbm.at[:, hs], k_v.at[:, hs], sem.at[s])

    def cp_v(g, s, n=1):
        hs = pl.ds(g * G, n * G)
        return pltpu.make_async_copy(v_hbm.at[:, hs], v_v.at[:, hs], sem.at[s])

    S_REST, S_OUT = NLOOP, NLOOP + 1

    def cp_out(r0, n, c0=0, nc=DM):
        rs, cs = pl.ds(r0, n), pl.ds(c0, nc)
        return pltpu.make_async_copy(out_v.at[rs, cs], out_hbm.at[rs, cs], sem.at[S_OUT])

    def cp_outt(r0, n):
        rs = pl.ds(r0, n)
        return pltpu.make_async_copy(outt_v.at[rs], out_hbm.at[rs, pl.ds(DM, D - DM)], sem.at[S_OUT])

    def set_copies(g):
        return [cp_wq(g + 2, g - 1), cp_k(g, g - 1), cp_v(g, g - 1), cp_wo(g - 1, g - 1)]

    gt = NLOOP + 1
    first = [[cp_wq_half(0, 0), cp_x(0, XR, 0)],
             [cp_wq_half(1, 1)],
             [cp_x(XR, XR, 2)],
             [cp_x(2 * XR, 2 * XR, 3)],
             [cp_wq(1, 4)],
             [cp_wq(2, 5), cp_k(0, 5), cp_v(0, 5)]]
    rest = [cp_wq(g, S_REST) for g in range(gt + 2, NG)]
    rest += [cp_k(gt, S_REST, NG - gt), cp_v(gt, S_REST, NG - gt)]
    rest += [cp_wo(g, S_REST) for g in range(gt - 1, NG)]

    def start(cps):
        for cp in cps:
            cp.start()

    def wait(cps):
        for cp in cps:
            cp.wait()

    for cps in first:
        start(cps)

    def Qtail(g, rows):
        qt_v[rows, :] = jnp.dot(x_v[rows, DM:D], wq_v[g, DM:D, :], preferred_element_type=f32)

    def Qtail_half(hf, r0, n):
        cs = slice(hf * (W // 2), (hf + 1) * (W // 2))
        for rr in (slice(r0, r0 + n // 2), slice(r0 + n // 2, r0 + n)):
            qt_v[rr, cs] = jnp.dot(x_v[rr, DM:D], wq_v[0, DM:D, cs], preferred_element_type=f32)

    def Qmain(g, j, rows):
        cs = slice(j * Dh, (j + 1) * Dh)
        q = jnp.dot(x_v[rows, 0:DM], wq_v[g, 0:DM, cs], preferred_element_type=f32)
        q_v[g, rows, cs] = (q + qt_v[rows, cs]).astype(bf)

    def QK(g, units, qc):
        res = []
        for b, j in units:
            qbh = qc[b * Sq:(b + 1) * Sq, j * Dh:(j + 1) * Dh]
            s = lax.dot_general(qbh, k_v[b, g * G + j], NT, preferred_element_type=f32)
            m = jnp.max(s, axis=-1, keepdims=True)
            p = jnp.exp2((s - m) * c)
            l = jnp.sum(p, axis=-1, keepdims=True)
            r = pl.reciprocal(l, approx=True)
            r = r * (2.0 - l * r)
            res.append((p * r).astype(bf))
        return res

    def PV(g, units, res, ohw):
        for n, (b, j) in enumerate(units):
            o = jnp.dot(res[n], v_v[b, g * G + j], preferred_element_type=f32)
            ohw[b * Sq:(b + 1) * Sq, j * Dh:(j + 1) * Dh] = o.astype(bf)

    def Omain(g, j, rows, ohp, final=False):
        cs = slice(j * 128, (j + 1) * 128)
        part = lax.dot_general(ohp[rows, :], wo_v[g, cs, :], NT, preferred_element_type=f32)
        if final:
            out_v[rows, cs] = (acc_v[rows, cs] + part).astype(bf)
        else:
            acc_v[rows, cs] += part

    def Otail(g, t, ohp, final=False):
        rows = slice(t * 128, (t + 1) * 128)
        part = lax.dot_general(wo_v[g, DM:D, :], ohp[rows, :], NT, preferred_element_type=f32)
        if final:
            outt_v[rows, :] = (tail_v[t] + part).T.astype(bf)
        else:
            tail_v[t] += part

    ALL = slice(0, M)
    H0, H1 = slice(0, M // 2), slice(M // 2, M)
    BY_HEAD = [[(b, i // 2) for b in range(4 * (i % 2), 4 * (i % 2) + 4)] for i in range(8)]
    BY_BATCH = [[(b, j) for j in range(G)] for b in range(B)]

    def attn_stage(g, qc, pos, ohw, order=BY_HEAD):
        res = None
        for n, units in enumerate(order):
            if res is not None:
                PV(g, order[n - 1], res, ohw)
            res = QK(g, units, qc)
            for f in pos[n]:
                f()
        PV(g, order[7], res, ohw)
        for f in pos[8]:
            f()

    def full_stage(g, qc, ohp, ohw):
        Qtail(g + 2, ALL)
        for j in range(NJ - 1):
            Omain(g - 1, j, ALL, ohp)
        for t in range(NTT):
            Otail(g - 1, t, ohp)
        pos = [[P(Omain, g - 1, NJ - 1, ALL, ohp)]]
        pos += [[P(Qmain, g + 2, j, r)] for j in range(G) for r in (H0, H1)]
        attn_stage(g, qc, pos, ohw)

    def zero_body(i, carry):
        acc_v[pl.ds(pl.multiple_of(i * 128, 128), 128), :] = jnp.zeros((128, DM), f32)
        tail_v[i] = jnp.zeros((D - DM, 128), f32)
        return carry
    lax.fori_loop(0, NTT, zero_body, 0)

    R0, R1, R23 = slice(0, XR), slice(XR, 2 * XR), slice(2 * XR, M)
    wait(first[0])
    Qtail_half(0, 0, XR)
    Qmain(0, 0, R0)
    Qmain(0, 1, R0)
    start(set_copies(1))
    wait(first[1])
    Qtail_half(1, 0, XR)
    Qmain(0, 2, R0)
    Qmain(0, 3, R0)
    start(set_copies(2))
    wait(first[2])
    Qtail(0, R1)
    for j in range(G):
        Qmain(0, j, R1)
    start(set_copies(3))
    wait(first[3])
    Qtail(0, R23)
    for j in range(G):
        Qmain(0, j, R23)
    start(set_copies(4))
    wait(first[4])
    Qtail(1, ALL)
    for j in range(G):
        Qmain(1, j, ALL)
    start(rest)
    wait(first[5])
    Qtail(2, H0)
    hl = [P(Qtail, 2, H1)] + [P(Qmain, 2, j, r) for j in range(G) for r in (H0, H1)]
    attn_stage(0, q_v.at[0], [[f] for f in hl], oh_v.at[0])

    def body(g, carry):
        wait(set_copies(g))
        full_stage(g, q_v[g], oh_v.at[0], oh_v.at[0])
        return carry
    lax.fori_loop(1, NLOOP + 1, body, 0)

    wait(rest)
    for g in range(gt, NG - 2):
        full_stage(g, q_v.at[g], oh_v.at[0 if g == gt else g - 1], oh_v.at[g])

    g = NG - 2
    ohp = oh_v.at[g - 1]
    hl = [P(Omain, g - 1, j, r, ohp) for j in range(NJ) for r in (H0, H1)]
    T = [P(Otail, g - 1, t, ohp) for t in range(NTT)]
    attn_stage(g, q_v.at[g], [[f] for f in hl[:4]] + [T] + [[f] for f in hl[4:]], oh_v.at[g])

    g = NG - 1
    ohp = oh_v.at[g - 1]
    ohl = oh_v.at[g]
    TR = [slice(t * 128, (t + 1) * 128) for t in range(NTT)]
    outs = []

    def emit(*a):
        outs.append(cp_out(*a))
        outs[-1].start()

    def emitt(*a):
        outs.append(cp_outt(*a))
        outs[-1].start()

    def o6(rows, js):
        return [P(Omain, g - 1, j, rows, ohp) for j in js]

    def t7(t):
        return [P(Otail, g, t, ohl, True)]

    def o7(t, js=range(NJ)):
        return [P(Omain, g, j, TR[t], ohl, True) for j in js]

    T6 = [P(Otail, g - 1, t, ohp) for t in range(NTT)]
    pos = [o6(H0, [0, 1]),
           o6(H0, [2]) + T6[:3],
           o6(H0, [3]) + T6[3:],
           t7(0) + o7(0) + [P(emit, 0, 128)],
           t7(1) + o7(1) + [P(emit, 128, 128)],
           t7(2) + o7(2) + [P(emit, 256, 128)],
           o6(H1, [0, 1]),
           o6(H1, [2, 3]) + t7(3) + o7(3) + [P(emit, 384, 128), P(emitt, 0, 256)],
           t7(4) + o7(4) + [P(emit, 512, 128), P(emitt, 256, 256)]]
    attn_stage(g, q_v.at[g], pos, ohl, order=BY_BATCH)
    for f in t7(5) + o7(5, [3, 2, 1]):
        f()
    emit(640, 128, 128, DM - 128)
    emitt(512, 256)
    for f in o7(5, [0]):
        f()
    emit(640, 128, 0, 128)
    wait(outs)


@jax.jit
def pallas_standalone__mha_block_cached__near_ridge_kernel(x, k_cache, v_cache, wq, wo):
    B, Sq, D = x.shape
    _, H, Sk, Dh = k_cache.shape
    assert (B, Sq, D, H, Sk, Dh) == (8, 96, 576, 32, 96, 128)
    M = B * Sq
    NG = H // G
    DM = (D // 128) * 128
    kern = functools.partial(_kernel, B=B, Sq=Sq, D=D, H=H, Dh=Dh, c=Dh ** -0.5 * math.log2(math.e))
    bf = jnp.bfloat16
    out = pl.pallas_call(
        kern,
        in_specs=[pl.BlockSpec(memory_space=pl.ANY)] * 5,
        out_specs=pl.BlockSpec(memory_space=pl.ANY),
        out_shape=jax.ShapeDtypeStruct((M, D), x.dtype),
        scratch_shapes=[
            pltpu.VMEM((M, D), bf),
            pltpu.VMEM((B, H, Sk, Dh), bf),
            pltpu.VMEM((B, H, Sk, Dh), bf),
            pltpu.VMEM((NG, D, G * Dh), bf),
            pltpu.VMEM((NG, D, G * Dh), bf),
            pltpu.VMEM((M, G * Dh), jnp.float32),
            pltpu.VMEM((NG, M, G * Dh), bf),
            pltpu.VMEM((NG, M, G * Dh), bf),
            pltpu.VMEM((M, DM), jnp.float32),
            pltpu.VMEM((M // 128, D - DM, 128), jnp.float32),
            pltpu.VMEM((M, DM), bf),
            pltpu.VMEM((M, D - DM), bf),
            pltpu.SemaphoreType.DMA((NSEM,)),
        ],
        compiler_params=pltpu.CompilerParams(vmem_limit_bytes=100 * 1024 * 1024),
    )(x.reshape(M, D), k_cache, v_cache, wq, wo.T)
    return out.reshape(B, Sq, D)
```

```python
import functools
import math

import jax
import jax.numpy as jnp
from jax import lax
import jax.experimental.pallas as pl
import jax.experimental.pallas.tpu as pltpu

NT = (((1,), (1,)), ((), ()))
G = 4
NLOOP = 4
NSEM = 5
P = functools.partial


def _kernel(x_hbm, k_hbm, v_hbm, wq_hbm, wo_hbm, out_hbm,
            x_v, k_v, v_v, wq_v, wo_v, qt_v, q_v, oh_v, acc_v, tail_v, out_v, outt_v, sem,
            *, B, Sq, D, H, Dh, c):
    NG = H // G
    W = G * Dh
    M = B * Sq
    DM = (D // 128) * 128
    NJ = DM // 128
    NTT = M // 128
    XR = M // 4
    f32 = jnp.float32
    bf = jnp.bfloat16

    def cp_x(r0, n, s):
        return pltpu.make_async_copy(x_hbm.at[pl.ds(r0, n)], x_v.at[pl.ds(r0, n)], sem.at[s])

    def cp_wq(g, s):
        return pltpu.make_async_copy(wq_hbm.at[:, pl.ds(g * W, W)], wq_v.at[g], sem.at[s])

    def cp_wq_half(hf, s):
        cs = pl.ds(hf * (W // 2), W // 2)
        return pltpu.make_async_copy(wq_hbm.at[:, cs], wq_v.at[0, :, cs], sem.at[s])

    def cp_wo(g, s):
        return pltpu.make_async_copy(wo_hbm.at[:, pl.ds(g * W, W)], wo_v.at[g], sem.at[s])

    def cp_k(g, s, n=1):
        hs = pl.ds(g * G, n * G)
        return pltpu.make_async_copy(k_hbm.at[:, hs], k_v.at[:, hs], sem.at[s])

    def cp_v(g, s, n=1):
        hs = pl.ds(g * G, n * G)
        return pltpu.make_async_copy(v_hbm.at[:, hs], v_v.at[:, hs], sem.at[s])

    S_REST, S_OUT = NLOOP, 0

    def cp_out(r0, n, c0=0, nc=DM):
        rs, cs = pl.ds(r0, n), pl.ds(c0, nc)
        return pltpu.make_async_copy(out_v.at[rs, cs], out_hbm.at[rs, cs], sem.at[S_OUT])

    def cp_outt(r0, n):
        rs = pl.ds(r0, n)
        return pltpu.make_async_copy(outt_v.at[rs], out_hbm.at[rs, pl.ds(DM, D - DM)], sem.at[S_OUT])

    def set_copies(g):
        return [cp_k(g, g), cp_v(g, g), cp_wq(g + 3, g), cp_wo(g, g)]

    gt = NLOOP
    first = [[cp_wq_half(0, 0), cp_x(0, XR, 0)],
             [cp_wq_half(1, 1)],
             [cp_x(XR, XR, 2)],
             [cp_x(2 * XR, 2 * XR, 3)],
             [cp_wq(1, 4), cp_wq(2, 4)]]
    rest = [cp_wq(g, S_REST) for g in range(gt + 3, NG)]
    rest += [cp_k(gt, S_REST, NG - gt), cp_v(gt, S_REST, NG - gt)]
    rest += [cp_wo(g, S_REST) for g in range(gt, NG)]

    def start(cps):
        for cp in cps:
            cp.start()

    def wait(cps):
        for cp in cps:
            cp.wait()

    for cps in first:
        start(cps)

    def Qtail(g, rows):
        qt_v[rows, :] = jnp.dot(x_v[rows, DM:D], wq_v[g, DM:D, :], preferred_element_type=f32)

    def Qtail_half(hf, r0, n):
        cs = slice(hf * (W // 2), (hf + 1) * (W // 2))
        for rr in (slice(r0, r0 + n // 2), slice(r0 + n // 2, r0 + n)):
            qt_v[rr, cs] = jnp.dot(x_v[rr, DM:D], wq_v[0, DM:D, cs], preferred_element_type=f32)

    def Qmain(g, j, rows):
        cs = slice(j * Dh, (j + 1) * Dh)
        q = jnp.dot(x_v[rows, 0:DM], wq_v[g, 0:DM, cs], preferred_element_type=f32)
        q_v[g, rows, cs] = (q + qt_v[rows, cs]).astype(bf)

    def QK(g, units, qc):
        res = []
        for b, j in units:
            qbh = qc[b * Sq:(b + 1) * Sq, j * Dh:(j + 1) * Dh]
            s = lax.dot_general(qbh, k_v[b, g * G + j], NT, preferred_element_type=f32)
            m = jnp.max(s, axis=-1, keepdims=True)
            p = jnp.exp2((s - m) * c)
            l = jnp.sum(p, axis=-1, keepdims=True)
            r = pl.reciprocal(l, approx=True)
            r = r * (2.0 - l * r)
            res.append((p * r).astype(bf))
        return res

    def PV(g, units, res, ohw):
        for n, (b, j) in enumerate(units):
            o = jnp.dot(res[n], v_v[b, g * G + j], preferred_element_type=f32)
            ohw[b * Sq:(b + 1) * Sq, j * Dh:(j + 1) * Dh] = o.astype(bf)

    def Omain(g, j, rows, ohp, final=False):
        cs = slice(j * 128, (j + 1) * 128)
        part = lax.dot_general(ohp[rows, :], wo_v[g, cs, :], NT, preferred_element_type=f32)
        if final:
            out_v[rows, cs] = (acc_v[rows, cs] + part).astype(bf)
        else:
            acc_v[rows, cs] += part

    def Otail(g, t, ohp, final=False):
        rows = slice(t * 128, (t + 1) * 128)
        part = lax.dot_general(wo_v[g, DM:D, :], ohp[rows, :], NT, preferred_element_type=f32)
        if final:
            outt_v[rows, :] = (tail_v[t] + part).T.astype(bf)
        else:
            tail_v[t] += part

    ALL = slice(0, M)
    H0, H1 = slice(0, M // 2), slice(M // 2, M)
    BY_HEAD = [[(b, i // 2) for b in range(4 * (i % 2), 4 * (i % 2) + 4)] for i in range(8)]
    BY_BATCH = [[(b, j) for j in range(G)] for b in range(B)]

    def attn_stage(g, qc, pos, ohw, order=BY_HEAD):
        res = None
        for n, units in enumerate(order):
            if res is not None:
                PV(g, order[n - 1], res, ohw)
            res = QK(g, units, qc)
            for f in pos[n]:
                f()
        PV(g, order[7], res, ohw)
        for f in pos[8]:
            f()

    def aq_stage(g, qc, ohw):
        Qtail(g + 3, H0)
        hl = [P(Qtail, g + 3, H1)] + [P(Qmain, g + 3, j, r) for j in range(G) for r in (H0, H1)]
        attn_stage(g, qc, [[f] for f in hl], ohw)

    def ao_stage(g):
        ohp = oh_v.at[g - 1]
        hl = [P(Omain, g - 1, j, r, ohp) for j in range(NJ) for r in (H0, H1)]
        T = [P(Otail, g - 1, t, ohp) for t in range(NTT)]
        attn_stage(g, q_v.at[g], [[f] for f in hl[:4]] + [T] + [[f] for f in hl[4:]], oh_v.at[g])

    def zero_body(i, carry):
        acc_v[pl.ds(pl.multiple_of(i * 128, 128), 128), :] = jnp.zeros((128, DM), f32)
        tail_v[i] = jnp.zeros((D - DM, 128), f32)
        return carry
    lax.fori_loop(0, NTT, zero_body, 0)

    R0, R1, R23 = slice(0, XR), slice(XR, 2 * XR), slice(2 * XR, M)
    wait(first[0])
    Qtail_half(0, 0, XR)
    Qmain(0, 0, R0)
    Qmain(0, 1, R0)
    start(set_copies(0))
    wait(first[1])
    Qtail_half(1, 0, XR)
    Qmain(0, 2, R0)
    Qmain(0, 3, R0)
    start(set_copies(1))
    wait(first[2])
    Qtail(0, R1)
    for j in range(G):
        Qmain(0, j, R1)
    start(set_copies(2))
    wait(first[3])
    Qtail(0, R23)
    for j in range(G):
        Qmain(0, j, R23)
    start(set_copies(3))
    wait(first[4])
    for g in (1, 2):
        Qtail(g, ALL)
        for j in range(G):
            Qmain(g, j, ALL)
    start(rest)

    def body(g, carry):
        wait(set_copies(g))
        oh = oh_v.at[0]
        aq_stage(g, q_v[g], oh)
        for j in range(NJ):
            Omain(g, j, ALL, oh)
            if j == 0:
                for t in range(NTT):
                    Otail(g, t, oh)
        return carry
    lax.fori_loop(0, NLOOP, body, 0)

    wait(rest)
    aq_stage(gt, q_v.at[gt], oh_v.at[gt])
    for g in range(gt + 1, NG - 1):
        ao_stage(g)

    g = NG - 1
    ohp = oh_v.at[g - 1]
    ohl = oh_v.at[g]
    TR = [slice(t * 128, (t + 1) * 128) for t in range(NTT)]
    outs = []

    def emit(*a):
        outs.append(cp_out(*a))
        outs[-1].start()

    def emitt(*a):
        outs.append(cp_outt(*a))
        outs[-1].start()

    def o6(rows, js):
        return [P(Omain, g - 1, j, rows, ohp) for j in js]

    def t7(t):
        return [P(Otail, g, t, ohl, True)]

    def o7(t, js=range(NJ)):
        return [P(Omain, g, j, TR[t], ohl, True) for j in js]

    T6 = [P(Otail, g - 1, t, ohp) for t in range(NTT)]
    pos = [o6(H0, [0, 1]),
           o6(H0, [2]) + T6[:3],
           o6(H0, [3]) + T6[3:],
           t7(0) + o7(0) + [P(emit, 0, 128)],
           t7(1) + o7(1) + [P(emit, 128, 128)],
           t7(2) + o7(2) + [P(emit, 256, 128)],
           o6(H1, [0, 1]),
           o6(H1, [2, 3]) + t7(3) + o7(3) + [P(emit, 384, 128), P(emitt, 0, 256)],
           t7(4) + o7(4) + [P(emit, 512, 128), P(emitt, 256, 256)]]
    attn_stage(g, q_v.at[g], pos, ohl, order=BY_BATCH)
    for f in t7(5) + o7(5, [3, 2, 1]):
        f()
    emit(640, 128, 128, DM - 128)
    emitt(512, 256)
    for f in o7(5, [0]):
        f()
    emit(640, 128, 0, 128)
    wait(outs)


@jax.jit
def pallas_standalone__mha_block_cached__near_ridge_kernel(x, k_cache, v_cache, wq, wo):
    B, Sq, D = x.shape
    _, H, Sk, Dh = k_cache.shape
    assert (B, Sq, D, H, Sk, Dh) == (8, 96, 576, 32, 96, 128)
    M = B * Sq
    NG = H // G
    DM = (D // 128) * 128
    kern = functools.partial(_kernel, B=B, Sq=Sq, D=D, H=H, Dh=Dh, c=Dh ** -0.5 * math.log2(math.e))
    bf = jnp.bfloat16
    out = pl.pallas_call(
        kern,
        in_specs=[pl.BlockSpec(memory_space=pl.ANY)] * 5,
        out_specs=pl.BlockSpec(memory_space=pl.ANY),
        out_shape=jax.ShapeDtypeStruct((M, D), x.dtype),
        scratch_shapes=[
            pltpu.VMEM((M, D), bf),
            pltpu.VMEM((B, H, Sk, Dh), bf),
            pltpu.VMEM((B, H, Sk, Dh), bf),
            pltpu.VMEM((NG, D, G * Dh), bf),
            pltpu.VMEM((NG, D, G * Dh), bf),
            pltpu.VMEM((M, G * Dh), jnp.float32),
            pltpu.VMEM((NG, M, G * Dh), bf),
            pltpu.VMEM((NG, M, G * Dh), bf),
            pltpu.VMEM((M, DM), jnp.float32),
            pltpu.VMEM((M // 128, D - DM, 128), jnp.float32),
            pltpu.VMEM((M, DM), bf),
            pltpu.VMEM((M, D - DM), bf),
            pltpu.SemaphoreType.DMA((NSEM,)),
        ],
        compiler_params=pltpu.CompilerParams(vmem_limit_bytes=100 * 1024 * 1024),
    )(x.reshape(M, D), k_cache, v_cache, wq, wo.T)
    return out.reshape(B, Sq, D)
```

```python
import functools
import math

import jax
import jax.numpy as jnp
from jax import lax
import jax.experimental.pallas as pl
import jax.experimental.pallas.tpu as pltpu

NT = (((1,), (1,)), ((), ()))
G = 4
NLOOP = 4
NSEM = 5
P = functools.partial


def _kernel(x_hbm, k_hbm, v_hbm, wq_hbm, wo_hbm, out_hbm,
            x_v, k_v, v_v, wq_v, wo_v, qt_v, q_v, oh_v, acc_v, tail_v, out_v, outt_v, sem,
            *, B, Sq, D, H, Dh, c):
    NG = H // G
    W = G * Dh
    M = B * Sq
    DM = (D // 128) * 128
    NJ = DM // 128
    NTT = M // 128
    XR = M // 4
    f32 = jnp.float32
    bf = jnp.bfloat16

    def cp_x(r0, n, s):
        return pltpu.make_async_copy(x_hbm.at[pl.ds(r0, n)], x_v.at[pl.ds(r0, n)], sem.at[s])

    def cp_wq(g, s):
        return pltpu.make_async_copy(wq_hbm.at[:, pl.ds(g * W, W)], wq_v.at[g], sem.at[s])

    KS = 256

    def cp_wq0(k0, n, s):
        return pltpu.make_async_copy(wq_hbm.at[pl.ds(k0, n), pl.ds(0, W)], wq_v.at[0, pl.ds(k0, n)], sem.at[s])

    def cp_wo(g, s):
        return pltpu.make_async_copy(wo_hbm.at[:, pl.ds(g * W, W)], wo_v.at[g], sem.at[s])

    def cp_k(g, s, n=1):
        hs = pl.ds(g * G, n * G)
        return pltpu.make_async_copy(k_hbm.at[:, hs], k_v.at[:, hs], sem.at[s])

    def cp_v(g, s, n=1):
        hs = pl.ds(g * G, n * G)
        return pltpu.make_async_copy(v_hbm.at[:, hs], v_v.at[:, hs], sem.at[s])

    S_REST, S_OUT = NLOOP, 0

    def cp_out(r0, n, c0=0, nc=DM):
        rs, cs = pl.ds(r0, n), pl.ds(c0, nc)
        return pltpu.make_async_copy(out_v.at[rs, cs], out_hbm.at[rs, cs], sem.at[S_OUT])

    def cp_outt(r0, n):
        rs = pl.ds(r0, n)
        return pltpu.make_async_copy(outt_v.at[rs], out_hbm.at[rs, pl.ds(DM, D - DM)], sem.at[S_OUT])

    def set_copies(g):
        return [cp_k(g, g), cp_v(g, g), cp_wq(g + 3, g), cp_wo(g, g)]

    gt = NLOOP
    first = [[cp_wq0(0, KS, 0), cp_x(0, XR, 0)],
             [cp_wq0(KS, D - KS, 1)],
             [cp_x(XR, XR, 2)],
             [cp_x(2 * XR, 2 * XR, 3)],
             [cp_wq(1, 4), cp_wq(2, 4)]]
    rest = [cp_wq(g, S_REST) for g in range(gt + 3, NG)]
    rest += [cp_k(gt, S_REST, NG - gt), cp_v(gt, S_REST, NG - gt)]
    rest += [cp_wo(g, S_REST) for g in range(gt, NG)]

    def start(cps):
        for cp in cps:
            cp.start()

    def wait(cps):
        for cp in cps:
            cp.wait()

    for cps in first:
        start(cps)

    def Qtail(g, rows):
        qt_v[rows, :] = jnp.dot(x_v[rows, DM:D], wq_v[g, DM:D, :], preferred_element_type=f32)

    def Qmain(g, j, rows):
        cs = slice(j * Dh, (j + 1) * Dh)
        q = jnp.dot(x_v[rows, 0:DM], wq_v[g, 0:DM, cs], preferred_element_type=f32)
        q_v[g, rows, cs] = (q + qt_v[rows, cs]).astype(bf)

    def QK(g, units, qc):
        res = []
        for b, j in units:
            qbh = qc[b * Sq:(b + 1) * Sq, j * Dh:(j + 1) * Dh]
            s = lax.dot_general(qbh, k_v[b, g * G + j], NT, preferred_element_type=f32)
            m = jnp.max(s, axis=-1, keepdims=True)
            p = jnp.exp2((s - m) * c)
            l = jnp.sum(p, axis=-1, keepdims=True)
            r = pl.reciprocal(l, approx=True)
            r = r * (2.0 - l * r)
            res.append((p * r).astype(bf))
        return res

    def PV(g, units, res, ohw):
        for n, (b, j) in enumerate(units):
            o = jnp.dot(res[n], v_v[b, g * G + j], preferred_element_type=f32)
            ohw[b * Sq:(b + 1) * Sq, j * Dh:(j + 1) * Dh] = o.astype(bf)

    def Omain(g, j, rows, ohp, final=False):
        cs = slice(j * 128, (j + 1) * 128)
        part = lax.dot_general(ohp[rows, :], wo_v[g, cs, :], NT, preferred_element_type=f32)
        if final:
            out_v[rows, cs] = (acc_v[rows, cs] + part).astype(bf)
        else:
            acc_v[rows, cs] += part

    def Otail(g, t, ohp, final=False):
        rows = slice(t * 128, (t + 1) * 128)
        part = lax.dot_general(wo_v[g, DM:D, :], ohp[rows, :], NT, preferred_element_type=f32)
        if final:
            outt_v[rows, :] = (tail_v[t] + part).T.astype(bf)
        else:
            tail_v[t] += part

    ALL = slice(0, M)
    H0, H1 = slice(0, M // 2), slice(M // 2, M)
    BY_HEAD = [[(b, i // 2) for b in range(4 * (i % 2), 4 * (i % 2) + 4)] for i in range(8)]
    BY_BATCH = [[(b, j) for j in range(G)] for b in range(B)]

    def attn_stage(g, qc, pos, ohw, order=BY_HEAD):
        res = None
        for n, units in enumerate(order):
            if res is not None:
                PV(g, order[n - 1], res, ohw)
            res = QK(g, units, qc)
            for f in pos[n]:
                f()
        PV(g, order[7], res, ohw)
        for f in pos[8]:
            f()

    def aq_stage(g, qc, ohw):
        Qtail(g + 3, H0)
        hl = [P(Qtail, g + 3, H1)] + [P(Qmain, g + 3, j, r) for j in range(G) for r in (H0, H1)]
        attn_stage(g, qc, [[f] for f in hl], ohw)

    def ao_stage(g):
        ohp = oh_v.at[g - 1]
        hl = [P(Omain, g - 1, j, r, ohp) for j in range(NJ) for r in (H0, H1)]
        T = [P(Otail, g - 1, t, ohp) for t in range(NTT)]
        attn_stage(g, q_v.at[g], [[f] for f in hl[:4]] + [T] + [[f] for f in hl[4:]], oh_v.at[g])

    def zero_body(i, carry):
        acc_v[pl.ds(pl.multiple_of(i * 128, 128), 128), :] = jnp.zeros((128, DM), f32)
        tail_v[i] = jnp.zeros((D - DM, 128), f32)
        return carry
    lax.fori_loop(0, NTT, zero_body, 0)

    R0, R1, R23 = slice(0, XR), slice(XR, 2 * XR), slice(2 * XR, M)
    wait(first[0])
    qt_v[R0, :] = jnp.dot(x_v[R0, 0:KS], wq_v[0, 0:KS, :], preferred_element_type=f32)
    start(set_copies(0))
    wait(first[1])
    q0 = jnp.dot(x_v[R0, KS:D], wq_v[0, KS:D, :], preferred_element_type=f32)
    q_v[0, R0, :] = (q0 + qt_v[R0, :]).astype(bf)
    start(set_copies(1))
    wait(first[2])
    Qtail(0, R1)
    for j in range(G):
        Qmain(0, j, R1)
    start(set_copies(2))
    wait(first[3])
    Qtail(0, R23)
    for j in range(G):
        Qmain(0, j, R23)
    start(set_copies(3))
    wait(first[4])
    for g in (1, 2):
        Qtail(g, ALL)
        for j in range(G):
            Qmain(g, j, ALL)
    start(rest)

    def body(g, carry):
        wait(set_copies(g))
        oh = oh_v.at[0]
        aq_stage(g, q_v[g], oh)
        for j in range(NJ):
            Omain(g, j, ALL, oh)
            if j == 0:
                for t in range(NTT):
                    Otail(g, t, oh)
        return carry
    lax.fori_loop(0, NLOOP, body, 0)

    wait(rest)
    aq_stage(gt, q_v.at[gt], oh_v.at[gt])
    for g in range(gt + 1, NG - 1):
        ao_stage(g)

    g = NG - 1
    ohp = oh_v.at[g - 1]
    ohl = oh_v.at[g]
    TR = [slice(t * 128, (t + 1) * 128) for t in range(NTT)]
    outs = []

    def emit(*a):
        outs.append(cp_out(*a))
        outs[-1].start()

    def emitt(*a):
        outs.append(cp_outt(*a))
        outs[-1].start()

    def o6(rows, js):
        return [P(Omain, g - 1, j, rows, ohp) for j in js]

    def t7(t):
        return [P(Otail, g, t, ohl, True)]

    def o7(t, js=range(NJ)):
        return [P(Omain, g, j, TR[t], ohl, True) for j in js]

    T6 = [P(Otail, g - 1, t, ohp) for t in range(NTT)]
    pos = [o6(H0, [0, 1]),
           o6(H0, [2]) + T6[:3],
           o6(H0, [3]) + T6[3:],
           t7(0) + o7(0) + [P(emit, 0, 128)],
           t7(1) + o7(1) + [P(emit, 128, 128)],
           t7(2) + o7(2) + [P(emit, 256, 128)],
           o6(H1, [0, 1]),
           o6(H1, [2, 3]) + t7(3) + o7(3) + [P(emit, 384, 128), P(emitt, 0, 256)],
           t7(4) + o7(4) + [P(emit, 512, 128), P(emitt, 256, 256)]]
    attn_stage(g, q_v.at[g], pos, ohl, order=BY_BATCH)
    for f in t7(5) + o7(5, [3, 2, 1]):
        f()
    emit(640, 128, 128, DM - 128)
    emitt(512, 256)
    for f in o7(5, [0]):
        f()
    emit(640, 128, 0, 128)
    wait(outs)


@jax.jit
def pallas_standalone__mha_block_cached__near_ridge_kernel(x, k_cache, v_cache, wq, wo):
    B, Sq, D = x.shape
    _, H, Sk, Dh = k_cache.shape
    assert (B, Sq, D, H, Sk, Dh) == (8, 96, 576, 32, 96, 128)
    M = B * Sq
    NG = H // G
    DM = (D // 128) * 128
    kern = functools.partial(_kernel, B=B, Sq=Sq, D=D, H=H, Dh=Dh, c=Dh ** -0.5 * math.log2(math.e))
    bf = jnp.bfloat16
    out = pl.pallas_call(
        kern,
        in_specs=[pl.BlockSpec(memory_space=pl.ANY)] * 5,
        out_specs=pl.BlockSpec(memory_space=pl.ANY),
        out_shape=jax.ShapeDtypeStruct((M, D), x.dtype),
        scratch_shapes=[
            pltpu.VMEM((M, D), bf),
            pltpu.VMEM((B, H, Sk, Dh), bf),
            pltpu.VMEM((B, H, Sk, Dh), bf),
            pltpu.VMEM((NG, D, G * Dh), bf),
            pltpu.VMEM((NG, D, G * Dh), bf),
            pltpu.VMEM((M, G * Dh), jnp.float32),
            pltpu.VMEM((NG, M, G * Dh), bf),
            pltpu.VMEM((NG, M, G * Dh), bf),
            pltpu.VMEM((M, DM), jnp.float32),
            pltpu.VMEM((M // 128, D - DM, 128), jnp.float32),
            pltpu.VMEM((M, DM), bf),
            pltpu.VMEM((M, D - DM), bf),
            pltpu.SemaphoreType.DMA((NSEM,)),
        ],
        compiler_params=pltpu.CompilerParams(vmem_limit_bytes=100 * 1024 * 1024),
    )(x.reshape(M, D), k_cache, v_cache, wq, wo.T)
    return out.reshape(B, Sq, D)
```
